```python
import os as _os
_os.environ.setdefault("JAX_PLATFORMS", "cpu")
import jax
import jax.numpy as jnp

def _softmax(x, axis=-1):
    return jax.nn.softmax(x, axis=axis)
def _gelu(x):
    return jax.nn.gelu(x, approximate=True)
def _silu(x):
    return jax.nn.silu(x)
def _sigmoid(x):
    return jax.nn.sigmoid(x)
def _layernorm(x, axis=-1, eps=1e-5):
    m = jnp.mean(x, axis=axis, keepdims=True)
    v = jnp.var(x, axis=axis, keepdims=True)
    return (x - m) / jnp.sqrt(v + eps)
def _scatter_add(tgt, idx, src, axis=0):
    return tgt.at[idx].add(src)
def _segment_sum(src, seg, n):
    return jax.ops.segment_sum(src, seg, n)
class _Rng:
    def __init__(self, key):
        self._k = key
    def _next(self):
        self._k, sub = jax.random.split(self._k)
        return sub
    def normal(self, shape):
        return jax.random.normal(self._next(), shape, dtype=jnp.bfloat16)
    def randint(self, lo, hi, shape):
        return jax.random.randint(self._next(), shape, lo, hi, dtype=jnp.int32)
    def uniform(self, shape, lo=0.0, hi=1.0):
        return jax.random.uniform(self._next(), shape, jnp.bfloat16, lo, hi)
    def permutation(self, n):
        return jax.random.permutation(self._next(), n)


kernel_name = 'standalone__seq2seq_rnn_t_joint__speech'

def setup_inputs():
    _rng = _Rng(jax.random.key(int.from_bytes(__import__("os").urandom(4), "little")))
    _w = (lambda a: (lambda t: t.astype(jnp.bfloat16) if jnp.issubdtype(t.dtype, jnp.floating) else t)(jnp.asarray(a)))
    B, T, D, K = 2, 1000, 512, 31
    U = 8
    sc = (1.0 / (K * D)) ** 0.5
    sd = (1.0 / D) ** 0.5
    return {
        "x": _w((lambda *s: _rng.normal(s) * 0.4)(B, T, D) * 0.5),
        "w1": _w((lambda *s: _rng.normal(s) * 1.6)(K, D, D) * sc),
        "w2": _w((lambda *s: _rng.normal(s) * 1.6)(K, D, D) * sc),
        "g": _w((lambda *s: _rng.normal(s) * 1.6)(B, U, D) * 0.5),
        "w_f": _w((lambda *s: _rng.normal(s) * 1.6)(D, D) * sd),
        "w_g": _w((lambda *s: _rng.normal(s) * 1.6)(D, D) * sd),
        "w_o": _w((lambda *s: _rng.normal(s) * 1.6)(D, D) * sd),
    }

def reference(x, w1, w2, g, w_f, w_g, w_o):
    B, T, D = x.shape
    K = w1.shape[0]
    pad = K // 2
    xp = jnp.pad(x, ((0,0),(pad,pad),(0,0)))
    h = jnp.zeros_like(x)
    for i in range(K):
        h = h + jnp.einsum("btc,cd->btd", xp[:, i:i+T, :], w1[i])
    h = _gelu(h)[:, ::2, :]
    T1 = h.shape[1]
    hp = jnp.pad(h, ((0,0),(pad,pad),(0,0)))
    f = jnp.zeros_like(h)
    for i in range(K):
        f = f + jnp.einsum("btc,cd->btd", hp[:, i:i+T1, :], w2[i])
    f = _gelu(f)[:, ::2, :]
    fe = jnp.einsum("btd,de->bte", f, w_f)
    ge = jnp.einsum("bud,de->bue", g, w_g)
    j = jnp.tanh(fe[:, :, None, :] + ge[:, None, :, :])
    return jnp.einsum("btud,dv->btuv", j, w_o)
```

```python
import functools
import itertools

import jax
import jax.numpy as jnp
import jax.experimental.pallas as pl
import jax.experimental.pallas.tpu as pltpu

F32 = jnp.float32
BF16 = jnp.bfloat16

B, T, D, K, U = 2, 1000, 512, 31, 8
PAD = K // 2
T1, T2 = T // 2, T // 4
A = 8
R = B * A
PV1, PV2 = 8, 4
Q1, Q2 = 16 * PV1, 16 * PV2
M1, M2 = R * PV1, R * PV2
XOFF = 16
XPITCH = Q1 + 1
XROWS = 1064
LT = 128
NCT = D // LT
HD = D // 2
NM = 8 * PV2
NSTEP = 8
NFLAGS = 32

COMBOS = list(itertools.product(range(3), repeat=3))
_WSET = {0: (0,), 1: (0, 1), 2: (1,)}
MULTI = [c for c in COMBOS if 1 in c]
MULTI_IDX = {c: i for i, c in enumerate(MULTI)}
CIDX = {c: i for i, c in enumerate(COMBOS)}
NC = len(COMBOS)


def _single_tap(c):
    return _WSET[c[0]][0] + 2 * _WSET[c[1]][0] + 4 * _WSET[c[2]][0]


def _cols(t):
    return slice(LT * t, LT * (t + 1))


def _half(hf):
    return slice(HD * hf, HD * (hf + 1))


def _gelu(x):
    c = 0.7978845608028654
    return 0.5 * x * (1.0 + jnp.tanh(c * (x + 0.044715 * (x * x * x))))


def _fir_in(seq, which=(0, 1, 2)):
    n = (len(seq) - 1) // 2
    out = {}
    if 0 in which:
        out[0] = [seq[2 * i] - seq[2 * i + 1] for i in range(n)]
    if 1 in which:
        out[1] = [seq[2 * i + 1] for i in range(n)]
    if 2 in which:
        out[2] = [seq[2 * i + 1] - seq[2 * i + 2] for i in range(n)]
    return out


def _output_transform(get_acc):
    p3 = {}
    for c1 in range(3):
        for c2 in range(3):
            m = get_acc((c1, c2, 1))
            p3[(c1, c2, 0)] = get_acc((c1, c2, 0)) + m
            p3[(c1, c2, 1)] = m - get_acc((c1, c2, 2))
    p2 = {}
    for c1 in range(3):
        for e3 in range(2):
            m = p3[(c1, 1, e3)]
            p2[(c1, 0, e3)] = p3[(c1, 0, e3)] + m
            p2[(c1, 1, e3)] = m - p3[(c1, 2, e3)]
    out = [None] * 8
    for e2 in range(2):
        for e3 in range(2):
            m = p2[(1, e2, e3)]
            out[0 + 2 * e2 + 4 * e3] = p2[(0, e2, e3)] + m
            out[1 + 2 * e2 + 4 * e3] = m - p2[(2, e2, e3)]
    return out


def _tap(s, d):
    return 16 * ((s % 4) // 2) + 2 * d + s % 2


def _interleave(parts, tasks):
    total = sum(c for c, _ in tasks) or 1
    n, done, ti = len(parts), 0, 0
    for i, part in enumerate(parts):
        part()
        while ti < len(tasks) and done * n < total * (i + 1) - (total if i + 1 < n else 0) * 0.5:
            done += tasks[ti][0]
            tasks[ti][1]()
            ti += 1
    for _, fn in tasks[ti:]:
        fn()


WR = 8


def _kernel(flags, x_hbm, w1_hbm, w2_hbm, g_hbm, wf_hbm, wg_hbm, wo_hbm, out_hbm,
            xb, xf, d1, acc1, wraw, vt0, vth, hs, d2, acc2, wsm, gv, gev, fb, fe, jb, ov,
            sem_x, sem_w, sem_s, sem_o):
    w_hbm = (w1_hbm, w2_hbm)
    flag_ctr = itertools.count()

    def block(fn):
        pl.when(flags[next(flag_ctr)] == 0)(fn)

    def x_copies(ct):
        return [pltpu.make_async_copy(x_hbm.at[:, :, _cols(ct)], xb.at[ct], sem_x.at[ct])]

    def w0_copies(kt):
        return [pltpu.make_async_copy(w1_hbm.at[_tap(0, d), _cols(kt), :],
                                      wraw.at[0, d, _cols(kt), :], sem_w.at[kt])
                for d in range(8)]

    def w_sem(s, hf):
        return sem_w.at[NCT + 2 * (s - 1) + hf]

    def w_start(s, hf):
        for d in range(8):
            if _tap(s, d) < K:
                pltpu.make_async_copy(w_hbm[s // 4].at[_tap(s, d), :, _half(hf)],
                                      wraw.at[s, d, :, _half(hf)], w_sem(s, hf)).start()

    def w_wait(s, hf):
        def one(d):
            pltpu.make_async_copy(w1_hbm.at[0, :, _half(hf)],
                                  wraw.at[s, d, :, _half(hf)], w_sem(s, hf)).wait()
        for d in range(7):
            one(d)
        if isinstance(s, int):
            if _tap(s, 7) < K:
                one(7)
        else:
            pl.when(s % 4 != 3)(functools.partial(one, 7))

    small_copies = [
        pltpu.make_async_copy(g_hbm, gv, sem_s.at[0]),
        pltpu.make_async_copy(wg_hbm, wsm.at[1], sem_s.at[1]),
        pltpu.make_async_copy(wf_hbm, wsm.at[0], sem_s.at[2]),
        pltpu.make_async_copy(wo_hbm, wsm.at[2], sem_s.at[3]),
    ]

    def wchunk(s, r0, hf, dst, dr0, dcols):
        rs = slice(r0, r0 + WR)
        d = [wraw[s, i, rs, _half(hf)].astype(F32) for i in range(8)]
        lv = {}
        for b2 in range(2):
            for b1 in range(2):
                lo, hi = d[4 * b2 + 2 * b1], d[4 * b2 + 2 * b1 + 1]
                lv[(0, b1, b2)], lv[(1, b1, b2)], lv[(2, b1, b2)] = lo, lo + hi, hi
        lw = {}
        for b2 in range(2):
            for c1 in range(3):
                lo, hi = lv[(c1, 0, b2)], lv[(c1, 1, b2)]
                lw[(c1, 0, b2)], lw[(c1, 1, b2)], lw[(c1, 2, b2)] = lo, lo + hi, hi
        for c1 in range(3):
            for c2 in range(3):
                lo, hi = lw[(c1, c2, 0)], lw[(c1, c2, 1)]
                for c3, v in ((0, lo), (1, lo + hi), (2, hi)):
                    if (c1, c2, c3) in MULTI_IDX:
                        dst[MULTI_IDX[(c1, c2, c3)], dr0:dr0 + WR, dcols] = v.astype(BF16)

    def w0_tasks(kt):
        return [(19, functools.partial(wchunk, 0, LT * kt + r0, hf, vt0[kt], r0, _half(hf)))
                for r0 in range(0, LT, WR) for hf in range(2)]

    def wh_tasks(s, hf):
        return [(19, functools.partial(wchunk, s, r0, hf, vth[hf], r0, slice(None)))
                for r0 in range(0, D, WR)]

    def in_win(get_y, d_ref, h, ct, r, c1):
        y = [get_y(8 * r + o) if (c1 != 1 or o % 2 == 1) and (c1, o) not in ((0, 14), (2, 0)) else None
             for o in range(15)]
        l1 = _fir_in(y, (c1,))[c1]
        l2 = _fir_in(l1)
        for c2 in range(3):
            l3 = _fir_in(l2[c2])
            for c3 in range(3):
                d_ref[ct][h, CIDX[(c1, c2, c3)], R * r:R * (r + 1), :] = l3[c3][0].astype(BF16)

    def in_tasks(get_y, d_ref, pv, h, ct):
        return [(16, functools.partial(in_win, get_y, d_ref, h, ct, r, c1))
                for r in range(pv + 1) for c1 in range(3)]

    def y1(h, ct):
        def get(i):
            m = 2 * i - PAD + h
            st = XOFF + m + (m // Q1) * (XPITCH - Q1)
            return jnp.concatenate(
                [xf[b, ct, pl.ds(st, A, stride=XPITCH), :] for b in range(B)], axis=0)
        return get

    def y2(h, ct):
        return lambda i: hs[2 * i + h, :, _cols(ct)]

    def xconv(b, ct, a):
        n = min(Q1, T - Q1 * a)
        xf[b, ct, XOFF + XPITCH * a:XOFF + XPITCH * a + n, :] = xb[ct, b, Q1 * a:Q1 * a + n, :].astype(F32)

    def xtasks(ct):
        out = [(16, functools.partial(xconv, b, ct, a)) for b in range(B) for a in range(A)]
        return out + in_tasks(y1(0, ct), d1, PV1, 0, ct)

    def x1tasks(ct):
        return in_tasks(y1(1, ct), d1, PV1, 1, ct)

    def e1a(n, r, b):
        outs = _output_transform(lambda c: acc1[n][CIDX[c], R * r + A * b:R * r + A * (b + 1), :])
        for e in range(8):
            hs[PAD + 8 * r + e, A * b:A * (b + 1), _cols(n)] = outs[e]

    def e1b(n, r, b):
        a_idx = jax.lax.broadcasted_iota(jnp.int32, (A, LT), 0)
        rows = slice(A * b, A * (b + 1))
        for e in range(8):
            m = 8 * r + e
            v = _gelu(hs[PAD + m, rows, _cols(n)])
            if Q2 * (A - 1) + m >= T1:
                v = jnp.where(a_idx == A - 1, 0.0, v)
            hs[PAD + m, rows, _cols(n)] = v
            if m < PAD:
                hs[PAD + Q2 + m, rows, _cols(n)] = jnp.where(a_idx == A - 1, 0.0, pltpu.roll(v, A - 1, 0))
            if m >= Q2 - PAD:
                hs[PAD + m - Q2, rows, _cols(n)] = jnp.where(a_idx == 0, 0.0, pltpu.roll(v, 1, 0))

    def e1_tasks(n, lag=3):
        units = [(r, b) for r in range(PV1) for b in range(B)]
        out = []
        for i in range(len(units) + lag):
            if i < len(units):
                out.append((14, functools.partial(e1a, n, *units[i])))
            if i >= lag:
                out.append((26, functools.partial(e1b, n, *units[i - lag])))
        for h in range(2):
            out += in_tasks(y2(h, n), d2, PV2, h, n)
        return out

    def e2(n, r):
        outs = _output_transform(lambda c: acc2[CIDX[c], R * r:R * (r + 1), _cols(n)])
        for e in range(8):
            m = 8 * r + e
            fb[n][R * m:R * (m + 1), :] = _gelu(outs[e]).astype(BF16)

    def e2_tasks(n):
        return [(70, functools.partial(e2, n, r)) for r in range(PV2)]

    def part0(c, kt):
        if c in MULTI_IDX:
            w = vt0[kt][MULTI_IDX[c]]
        else:
            w = wraw[0, _single_tap(c), _cols(kt), :]
        p = jnp.dot(d1[kt][0, CIDX[c], 0:M1, :], w, preferred_element_type=F32)
        for n in range(NCT):
            if kt == 0:
                acc1[n][CIDX[c]] = p[:, _cols(n)]
            else:
                acc1[n][CIDX[c]] += p[:, _cols(n)]

    def part(conv, s, c, n):
        d_ref, m_rows = ((d1, M1), (d2, M2))[conv]
        if c in MULTI_IDX:
            w = vth[n // 2][MULTI_IDX[c], :, _cols(n % 2)]
        else:
            w = wraw[s, _single_tap(c), :, _cols(n)]
        r0 = pl.multiple_of(((s % 4) // 2) * R, R)
        lhs = jnp.concatenate([d_ref[ct][s % 2, CIDX[c], pl.ds(r0, m_rows), :] for ct in range(NCT)], axis=1)
        p = jnp.dot(lhs, w, preferred_element_type=F32)
        if conv == 0:
            acc1[n][CIDX[c]] += p
        else:
            acc2[CIDX[c], :, _cols(n)] += p

    def parts(conv, s, n):
        return [functools.partial(part, conv, s, c, n) for c in COMBOS]

    def jbuild(b, a, m0):
        geb = gev[U * b:U * (b + 1), :]
        js = []
        for m in range(m0, m0 + 2):
            frow = fe[pl.ds(R * m + A * b + a, 1), :]
            js.append(jnp.tanh(jnp.broadcast_to(frow, (U, D)) + geb))
        jb[b][U * m0:U * (m0 + 2), :] = jnp.concatenate(js, axis=0).astype(BF16)

    def jtasks(b, a, nt=NM):
        return [(8, functools.partial(jbuild, b, a, m0)) for m0 in range(0, nt, 2)]

    def out_copy(b, a, nt):
        r0 = U * NM * a if isinstance(a, int) else pl.multiple_of(U * NM * a, U * NM)
        rows = pl.ds(r0, U * nt)
        return pltpu.make_async_copy(ov.at[b, rows, :], out_hbm.at[b, rows, :], sem_o.at[A * b + a])

    def jpart(b, a, nt, n):
        r0 = U * NM * a if isinstance(a, int) else pl.multiple_of(U * NM * a, U * NM)
        o = jnp.dot(jb[b][0:U * nt, :], wsm[2, :, _cols(n)], preferred_element_type=F32)
        ov[b, pl.ds(r0, U * nt), _cols(n)] = o.astype(BF16)
        if n == NCT - 1:
            out_copy(b, a, nt).start()

    def jparts(b, a, nt=NM):
        return [functools.partial(jpart, b, a, nt, n) for n in range(NCT)]

    def fe_part(kt):
        p = jnp.dot(fb[kt][...], wsm[0, _cols(kt), :], preferred_element_type=F32)
        if kt == 0:
            fe[...] = p
        else:
            fe[...] += p

    groups = iter([(s, hf) for s in range(1, NSTEP) for hf in range(2)])

    def start_next():
        w_start(*next(groups))

    for kt in range(2):
        for cp in x_copies(kt) + w0_copies(kt):
            cp.start()

    def init():
        tail0 = XOFF + XPITCH * (A - 1) + T - Q1 * (A - 1)
        for b in range(B):
            for ct in range(NCT):
                xf[b, ct, 0:XOFF, :] = jnp.zeros((XOFF, LT), F32)
                xf[b, ct, tail0:XROWS, :] = jnp.zeros((XROWS - tail0, LT), F32)
        for s in (3, 7):
            wraw[s, 7] = jnp.zeros((D, D), BF16)
        acc2[...] = jnp.zeros(acc2.shape, F32)
    block(init)

    for cp in x_copies(0) + w0_copies(0):
        cp.wait()
    for cp in x_copies(2) + w0_copies(2):
        cp.start()

    def prep0():
        for _, fn in xtasks(0) + w0_tasks(0):
            fn()
    block(prep0)

    for kt in range(NCT):
        p0 = [functools.partial(part0, c, kt) for c in COMBOS]
        block(functools.partial(_interleave, p0[:NC // 3], x1tasks(kt - 1) if kt else []))
        if kt + 1 < NCT:
            for cp in x_copies(kt + 1) + w0_copies(kt + 1):
                cp.wait()
            if kt == 0:
                for cp in x_copies(3) + w0_copies(3):
                    cp.start()
            else:
                start_next()
            if kt == 2:
                start_next()
            tasks = xtasks(kt + 1) + w0_tasks(kt + 1)
        else:
            w_wait(1, 0)
            for _ in range(4):
                start_next()
            tasks = wh_tasks(1, 0) + x1tasks(NCT - 1)
        block(functools.partial(_interleave, p0[NC // 3:], tasks))

    def conv_loop(conv, lo, hi):
        fl = [next(flag_ctr) for _ in range(2)]

        def tile(s, n, last=False):
            wt = wh_tasks(s, 1) if n < 2 else wh_tasks(jnp.minimum(s + 1, NSTEP - 1), 0)
            wt = wt[:len(wt) // 2] if n % 2 == 0 else wt[len(wt) // 2:]
            if last:
                _interleave(parts(conv, s, n)[:-1], wt + e1_tasks(n - 1))
            else:
                _interleave(parts(conv, s, n), wt)

        def tiles(s, n0, n1):
            for n in range(n0, n1):
                tile(s, n)

        def blk_a(s):
            if conv == 0:
                pl.when(flags[fl[0]] == 0)(functools.partial(tile, s, 0))
                pl.when(s != hi - 1)(functools.partial(tile, s, 1))
                pl.when(s == hi - 1)(functools.partial(tile, s, 1, True))
            else:
                pl.when(flags[fl[0]] == 0)(functools.partial(tiles, s, 0, 2))

        def blk_b(s):
            if conv == 0:
                pl.when(s != hi - 1)(functools.partial(tiles, s, 2, 4))
                pl.when(s == hi - 1)(functools.partial(tile, s, 2, True))
                pl.when(s + flags[fl[1]] == hi - 1)(functools.partial(tile, s, 3, True))
            else:
                pl.when(flags[fl[1]] == 0)(functools.partial(tiles, s, 2, 4))

        later = [(j, hf, next(groups)) for j in range(lo, hi) for hf in range(2)] if conv == 0 else []

        def start_later(s, hf):
            for j, hf_j, grp in later:
                if hf_j == hf:
                    pl.when(s == j)(functools.partial(w_start, *grp))

        def body(s, carry):
            w_wait(s, 1)
            start_later(s, 0)
            blk_a(s)
            if conv == 0:
                w_wait(s + 1, 0)
                start_later(s, 1)
            else:
                pl.when(s + 1 < NSTEP)(lambda: w_wait(jnp.minimum(s + 1, NSTEP - 1), 0))
            blk_b(s)
            return carry

        jax.lax.fori_loop(lo, hi, body, 0)

    conv_loop(0, 1, 4)

    start_next()
    assert next(groups, None) is None
    for cp in small_copies:
        cp.start()

    def mid():
        for _, fn in e1_tasks(NCT - 1):
            fn()
    block(mid)

    conv_loop(1, 4, NSTEP)

    for cp in small_copies:
        cp.wait()

    def proj():
        gev[...] = jnp.dot(gv[...], wsm[1], preferred_element_type=F32)
        for _, fn in e2_tasks(0):
            fn()
        for kt in range(NCT):
            _interleave([functools.partial(fe_part, kt)], e2_tasks(kt + 1) if kt + 1 < NCT else [])
        for _, fn in jtasks(0, 0):
            fn()
    block(proj)

    def jbody(a, carry):
        _interleave(jparts(0, a), jtasks(1, a))
        _interleave(jparts(1, a), jtasks(0, a + 1))
        return carry
    jax.lax.fori_loop(0, A - 1, jbody, 0)

    nt_last = T2 - NM * (A - 1)

    def jtail():
        _interleave(jparts(0, A - 1, nt_last), jtasks(1, A - 1, nt_last))
        for p in jparts(1, A - 1, nt_last):
            p()
    block(jtail)

    for b in range(B):
        for a in range(A):
            out_copy(b, a, NM if a + 1 < A else nt_last).wait()
    assert next(flag_ctr) <= NFLAGS


@jax.jit
def pallas_standalone__seq2seq_rnn_t_joint__speech_kernel(
    x: jax.Array,
    w1: jax.Array,
    w2: jax.Array,
    g: jax.Array,
    w_f: jax.Array,
    w_g: jax.Array,
    w_o: jax.Array,
):
    any_spec = pl.BlockSpec(memory_space=pl.ANY)
    out = pl.pallas_call(
        _kernel,
        out_shape=jax.ShapeDtypeStruct((B, T2 * U, D), BF16),
        in_specs=[pl.BlockSpec(memory_space=pltpu.SMEM)] + [any_spec] * 7,
        out_specs=any_spec,
        scratch_shapes=[
            pltpu.VMEM((NCT, B, T, LT), BF16),
            pltpu.VMEM((B, NCT, XROWS, LT), F32),
            [pltpu.VMEM((2, NC, R * (PV1 + 1), LT), BF16)] * NCT,
            [pltpu.VMEM((NC, M1, LT), F32)] * NCT,
            pltpu.VMEM((NSTEP, 8, D, D), BF16),
            [pltpu.VMEM((len(MULTI), LT, D), BF16)] * NCT,
            [pltpu.VMEM((len(MULTI), D, HD), BF16)] * 2,
            pltpu.VMEM((Q2 + 2 * PAD, R, D), F32),
            [pltpu.VMEM((2, NC, R * (PV2 + 1), LT), BF16)] * NCT,
            pltpu.VMEM((NC, M2, D), F32),
            pltpu.VMEM((3, D, D), BF16),
            pltpu.VMEM((B * U, D), BF16),
            pltpu.VMEM((B * U, D), F32),
            [pltpu.VMEM((R * NM, LT), BF16)] * NCT,
            pltpu.VMEM((R * NM, D), F32),
            [pltpu.VMEM((U * NM, D), BF16)] * B,
            pltpu.VMEM((B, T2 * U, D), BF16),
            pltpu.SemaphoreType.DMA((NCT,)),
            pltpu.SemaphoreType.DMA((NCT + 2 * (NSTEP - 1),)),
            pltpu.SemaphoreType.DMA((4,)),
            pltpu.SemaphoreType.DMA((B * A,)),
        ],
        compiler_params=pltpu.CompilerParams(vmem_limit_bytes=120 * 1024 * 1024),
    )(jnp.zeros((NFLAGS,), jnp.int32), x, w1, w2, g.reshape(B * U, D), w_f, w_g, w_o)
    return out.reshape(B, T2, U, D)
```

```python
import functools
import itertools

import jax
import jax.numpy as jnp
import jax.experimental.pallas as pl
import jax.experimental.pallas.tpu as pltpu

F32 = jnp.float32
BF16 = jnp.bfloat16

B, T, D, K, U = 2, 1000, 512, 31, 8
PAD = K // 2
T1, T2 = T // 2, T // 4
A = 8
R = B * A
PV1, PV2 = 8, 4
Q1, Q2 = 16 * PV1, 16 * PV2
M1, M2 = R * PV1, R * PV2
XOFF = 16
XPITCH = Q1 + 1
XROWS = 1064
LT = 128
NCT = D // LT
HD = D // 2
NM = 8 * PV2
NSTEP = 8
NFLAGS = 32
S0_SPLIT = (9, 9, 9, 9)

COMBOS = list(itertools.product(range(3), repeat=3))
_WSET = {0: (0,), 1: (0, 1), 2: (1,)}
MULTI = [c for c in COMBOS if 1 in c]
MULTI_IDX = {c: i for i, c in enumerate(MULTI)}
CIDX = {c: i for i, c in enumerate(COMBOS)}
NC = len(COMBOS)


def _single_tap(c):
    return _WSET[c[0]][0] + 2 * _WSET[c[1]][0] + 4 * _WSET[c[2]][0]


def _cols(t):
    return slice(LT * t, LT * (t + 1))


def _half(hf):
    return slice(HD * hf, HD * (hf + 1))


def _gelu(x):
    c = 0.7978845608028654
    return 0.5 * x * (1.0 + jnp.tanh(c * (x + 0.044715 * (x * x * x))))


def _fir_in(seq, which=(0, 1, 2)):
    n = (len(seq) - 1) // 2
    out = {}
    if 0 in which:
        out[0] = [seq[2 * i] - seq[2 * i + 1] for i in range(n)]
    if 1 in which:
        out[1] = [seq[2 * i + 1] for i in range(n)]
    if 2 in which:
        out[2] = [seq[2 * i + 1] - seq[2 * i + 2] for i in range(n)]
    return out


def _output_transform(get_acc):
    p3 = {}
    for c1 in range(3):
        for c2 in range(3):
            m = get_acc((c1, c2, 1))
            p3[(c1, c2, 0)] = get_acc((c1, c2, 0)) + m
            p3[(c1, c2, 1)] = m - get_acc((c1, c2, 2))
    p2 = {}
    for c1 in range(3):
        for e3 in range(2):
            m = p3[(c1, 1, e3)]
            p2[(c1, 0, e3)] = p3[(c1, 0, e3)] + m
            p2[(c1, 1, e3)] = m - p3[(c1, 2, e3)]
    out = [None] * 8
    for e2 in range(2):
        for e3 in range(2):
            m = p2[(1, e2, e3)]
            out[0 + 2 * e2 + 4 * e3] = p2[(0, e2, e3)] + m
            out[1 + 2 * e2 + 4 * e3] = m - p2[(2, e2, e3)]
    return out


def _tap(s, d):
    return 16 * ((s % 4) // 2) + 2 * d + s % 2


def _interleave(parts, tasks):
    total = sum(c for c, _ in tasks) or 1
    n, done, ti = len(parts), 0, 0
    for i, part in enumerate(parts):
        part()
        while ti < len(tasks) and done * n < total * (i + 1) - (total if i + 1 < n else 0) * 0.5:
            done += tasks[ti][0]
            tasks[ti][1]()
            ti += 1
    for _, fn in tasks[ti:]:
        fn()


WR = 8


def _kernel(flags, x_hbm, w1_hbm, w2_hbm, g_hbm, wf_hbm, wg_hbm, wo_hbm, out_hbm,
            xb, xf, d1, acc1, wraw, vt0, vth, hs, d2, acc2, wsm, gv, gev, fb, fe, jb, ov,
            sem_x, sem_w, sem_s, sem_o):
    w_hbm = (w1_hbm, w2_hbm)
    flag_ctr = itertools.count()

    def block(fn):
        pl.when(flags[next(flag_ctr)] == 0)(fn)

    def x_copies(ct):
        return [pltpu.make_async_copy(x_hbm.at[:, :, _cols(ct)], xb.at[ct], sem_x.at[ct])]

    def w0_copies(kt):
        return [pltpu.make_async_copy(w1_hbm.at[_tap(0, d), _cols(kt), :],
                                      wraw.at[0, d, _cols(kt), :], sem_w.at[kt])
                for d in range(8)]

    def w_sem(s, hf):
        return sem_w.at[NCT + 2 * (s - 1) + hf]

    def w_start(s, hf):
        for d in range(8):
            if _tap(s, d) < K:
                pltpu.make_async_copy(w_hbm[s // 4].at[_tap(s, d), :, _half(hf)],
                                      wraw.at[s, d, :, _half(hf)], w_sem(s, hf)).start()

    def w_wait(s, hf):
        def one(d):
            pltpu.make_async_copy(w1_hbm.at[0, :, _half(hf)],
                                  wraw.at[s, d, :, _half(hf)], w_sem(s, hf)).wait()
        for d in range(7):
            one(d)
        if isinstance(s, int):
            if _tap(s, 7) < K:
                one(7)
        else:
            pl.when(s % 4 != 3)(functools.partial(one, 7))

    small_copies = [
        pltpu.make_async_copy(g_hbm, gv, sem_s.at[0]),
        pltpu.make_async_copy(wg_hbm, wsm.at[1], sem_s.at[1]),
        pltpu.make_async_copy(wf_hbm, wsm.at[0], sem_s.at[2]),
        pltpu.make_async_copy(wo_hbm, wsm.at[2], sem_s.at[3]),
    ]

    def wsums(d):
        lv = {}
        for b2 in range(2):
            for b1 in range(2):
                lo, hi = d[4 * b2 + 2 * b1], d[4 * b2 + 2 * b1 + 1]
                lv[(0, b1, b2)], lv[(1, b1, b2)], lv[(2, b1, b2)] = lo, lo + hi, hi
        lw = {}
        for b2 in range(2):
            for c1 in range(3):
                lo, hi = lv[(c1, 0, b2)], lv[(c1, 1, b2)]
                lw[(c1, 0, b2)], lw[(c1, 1, b2)], lw[(c1, 2, b2)] = lo, lo + hi, hi
        for c1 in range(3):
            for c2 in range(3):
                lo, hi = lw[(c1, c2, 0)], lw[(c1, c2, 1)]
                for c3, v in ((0, lo), (1, lo + hi), (2, hi)):
                    if (c1, c2, c3) in MULTI_IDX:
                        yield (c1, c2, c3), v

    def wchunk0(kt, r0, hf):
        rs = slice(LT * kt + r0, LT * kt + r0 + WR)
        for c, v in wsums([wraw[0, i, rs, _half(hf)].astype(F32) for i in range(8)]):
            vt0[kt][MULTI_IDX[c], r0:r0 + WR, _half(hf)] = v.astype(BF16)

    def wchunk(s, r0, n):
        rs = slice(r0, r0 + 2 * WR)
        for c, v in wsums([wraw[s, i, rs, _cols(n)].astype(F32) for i in range(8)]):
            vth[n][MULTI_IDX[c], rs, :] = v.astype(BF16)

    def w0_tasks(kt):
        return [(19, functools.partial(wchunk0, kt, r0, hf))
                for r0 in range(0, LT, WR) for hf in range(2)]

    def wh_tasks(s, hf):
        return [(19, functools.partial(wchunk, s, r0, n))
                for r0 in range(0, D, 2 * WR) for n in (2 * hf, 2 * hf + 1)]

    def in_win(get_y, d_ref, h, ct, r, c1):
        y = [get_y(8 * r + o) if (c1 != 1 or o % 2 == 1) and (c1, o) not in ((0, 14), (2, 0)) else None
             for o in range(15)]
        l1 = _fir_in(y, (c1,))[c1]
        l2 = _fir_in(l1)
        for c2 in range(3):
            l3 = _fir_in(l2[c2])
            for c3 in range(3):
                d_ref[ct][h, CIDX[(c1, c2, c3)], R * r:R * (r + 1), :] = l3[c3][0].astype(BF16)

    def in_tasks(get_y, d_ref, pv, h, ct):
        return [(16, functools.partial(in_win, get_y, d_ref, h, ct, r, c1))
                for r in range(pv + 1) for c1 in range(3)]

    def y1(h, ct):
        def get(i):
            m = 2 * i - PAD + h
            st = XOFF + m + (m // Q1) * (XPITCH - Q1)
            return jnp.concatenate(
                [xf[b, ct, pl.ds(st, A, stride=XPITCH), :] for b in range(B)], axis=0)
        return get

    def y2(h, ct):
        return lambda i: hs[2 * i + h, :, _cols(ct)]

    def xconv(b, ct, a):
        n = min(Q1, T - Q1 * a)
        xf[b, ct, XOFF + XPITCH * a:XOFF + XPITCH * a + n, :] = xb[ct, b, Q1 * a:Q1 * a + n, :].astype(F32)

    def xtasks(ct):
        out = [(16, functools.partial(xconv, b, ct, a)) for b in range(B) for a in range(A)]
        return out + in_tasks(y1(0, ct), d1, PV1, 0, ct)

    def x1tasks(ct):
        return in_tasks(y1(1, ct), d1, PV1, 1, ct)

    def e1a(n, r, b):
        outs = _output_transform(lambda c: acc1[n][CIDX[c], R * r + A * b:R * r + A * (b + 1), :])
        for e in range(8):
            hs[PAD + 8 * r + e, A * b:A * (b + 1), _cols(n)] = outs[e]

    def e1b(n, r, b):
        a_idx = jax.lax.broadcasted_iota(jnp.int32, (A, LT), 0)
        rows = slice(A * b, A * (b + 1))
        for e in range(8):
            m = 8 * r + e
            v = _gelu(hs[PAD + m, rows, _cols(n)])
            if Q2 * (A - 1) + m >= T1:
                v = jnp.where(a_idx == A - 1, 0.0, v)
            hs[PAD + m, rows, _cols(n)] = v
            if m < PAD:
                hs[PAD + Q2 + m, rows, _cols(n)] = jnp.where(a_idx == A - 1, 0.0, pltpu.roll(v, A - 1, 0))
            if m >= Q2 - PAD:
                hs[PAD + m - Q2, rows, _cols(n)] = jnp.where(a_idx == 0, 0.0, pltpu.roll(v, 1, 0))

    def e1_tasks(n, lag=3):
        units = [(r, b) for r in range(PV1) for b in range(B)]
        out = []
        for i in range(len(units) + lag):
            if i < len(units):
                out.append((14, functools.partial(e1a, n, *units[i])))
            if i >= lag:
                out.append((26, functools.partial(e1b, n, *units[i - lag])))
        for h in range(2):
            out += in_tasks(y2(h, n), d2, PV2, h, n)
        return out

    def e2(n, r):
        outs = _output_transform(lambda c: acc2[CIDX[c], R * r:R * (r + 1), _cols(n)])
        for e in range(8):
            m = 8 * r + e
            fb[n][R * m:R * (m + 1), :] = _gelu(outs[e]).astype(BF16)

    def e2_tasks(n):
        return [(70, functools.partial(e2, n, r)) for r in range(PV2)]

    def part0(c, kt):
        if c in MULTI_IDX:
            w = vt0[kt][MULTI_IDX[c]]
        else:
            w = wraw[0, _single_tap(c), _cols(kt), :]
        p = jnp.dot(d1[kt][0, CIDX[c], 0:M1, :], w, preferred_element_type=F32)
        for n in range(NCT):
            if kt == 0:
                acc1[n][CIDX[c]] = p[:, _cols(n)]
            else:
                acc1[n][CIDX[c]] += p[:, _cols(n)]

    def part(conv, s, c, n):
        d_ref, m_rows = ((d1, M1), (d2, M2))[conv]
        if c in MULTI_IDX:
            w = vth[n][MULTI_IDX[c]]
        else:
            w = wraw[s, _single_tap(c), :, _cols(n)]
        r0 = pl.multiple_of(((s % 4) // 2) * R, R)
        lhs = jnp.concatenate([d_ref[ct][s % 2, CIDX[c], pl.ds(r0, m_rows), :] for ct in range(NCT)], axis=1)
        p = jnp.dot(lhs, w, preferred_element_type=F32)
        if conv == 0:
            acc1[n][CIDX[c]] += p
        else:
            acc2[CIDX[c], :, _cols(n)] += p

    def parts(conv, s, n):
        return [functools.partial(part, conv, s, c, n) for c in COMBOS]

    def jbuild(b, a, m0):
        geb = gev[U * b:U * (b + 1), :]
        js = []
        for m in range(m0, m0 + 2):
            frow = fe[pl.ds(R * m + A * b + a, 1), :]
            js.append(jnp.tanh(jnp.broadcast_to(frow, (U, D)) + geb))
        jb[b][U * m0:U * (m0 + 2), :] = jnp.concatenate(js, axis=0).astype(BF16)

    def jtasks(b, a, nt=NM):
        return [(8, functools.partial(jbuild, b, a, m0)) for m0 in range(0, nt, 2)]

    def out_copy(b, a, nt):
        r0 = U * NM * a if isinstance(a, int) else pl.multiple_of(U * NM * a, U * NM)
        rows = pl.ds(r0, U * nt)
        return pltpu.make_async_copy(ov.at[b, rows, :], out_hbm.at[b, rows, :], sem_o.at[A * b + a])

    def jpart(b, a, nt, n):
        r0 = U * NM * a if isinstance(a, int) else pl.multiple_of(U * NM * a, U * NM)
        o = jnp.dot(jb[b][0:U * nt, :], wsm[2, :, _cols(n)], preferred_element_type=F32)
        ov[b, pl.ds(r0, U * nt), _cols(n)] = o.astype(BF16)
        if n == NCT - 1:
            out_copy(b, a, nt).start()

    def jparts(b, a, nt=NM):
        return [functools.partial(jpart, b, a, nt, n) for n in range(NCT)]

    def fe_part(kt):
        p = jnp.dot(fb[kt][...], wsm[0, _cols(kt), :], preferred_element_type=F32)
        if kt == 0:
            fe[...] = p
        else:
            fe[...] += p

    groups = iter([(s, hf) for s in range(1, NSTEP) for hf in range(2)])

    def start_next():
        w_start(*next(groups))

    for cp in x_copies(0) + w0_copies(0):
        cp.start()

    def init():
        tail0 = XOFF + XPITCH * (A - 1) + T - Q1 * (A - 1)
        for b in range(B):
            for ct in range(NCT):
                xf[b, ct, 0:XOFF, :] = jnp.zeros((XOFF, LT), F32)
                xf[b, ct, tail0:XROWS, :] = jnp.zeros((XROWS - tail0, LT), F32)
        for s in (3, 7):
            wraw[s, 7] = jnp.zeros((D, D), BF16)
        acc2[...] = jnp.zeros(acc2.shape, F32)
    block(init)
    for cp in x_copies(1) + w0_copies(1):
        cp.start()

    for cp in x_copies(0):
        cp.wait()

    def prep0():
        for _, fn in xtasks(0):
            fn()
    block(prep0)
    for cp in w0_copies(0):
        cp.wait()
    for cp in x_copies(2) + w0_copies(2):
        cp.start()

    for kt in range(NCT):
        order = [c for c in COMBOS if c not in MULTI_IDX] + MULTI if kt == 0 else COMBOS
        p0 = [functools.partial(part0, c, kt) for c in order]
        sp = S0_SPLIT[kt]
        if kt == 0:
            block(lambda p0=p0, sp=sp: (_interleave(p0[:NC - len(MULTI)], w0_tasks(0)),
                                        _interleave(p0[NC - len(MULTI):sp], [])) and None)
        else:
            block(functools.partial(_interleave, p0[:sp], x1tasks(kt - 1)))
        if kt + 1 < NCT:
            for cp in x_copies(kt + 1) + w0_copies(kt + 1):
                cp.wait()
            if kt == 0:
                for cp in x_copies(3) + w0_copies(3):
                    cp.start()
            else:
                start_next()
            if kt == 2:
                start_next()
            tasks = xtasks(kt + 1) + w0_tasks(kt + 1)
        else:
            w_wait(1, 0)
            for _ in range(4):
                start_next()
            tasks = wh_tasks(1, 0) + x1tasks(NCT - 1)
        block(functools.partial(_interleave, p0[sp:], tasks))

    def conv_loop(conv, lo, hi):
        fl = [next(flag_ctr) for _ in range(2)]

        def tile(s, n, last=False):
            wt = wh_tasks(s, 1) if n < 2 else wh_tasks(jnp.minimum(s + 1, NSTEP - 1), 0)
            wt = wt[:len(wt) // 2] if n % 2 == 0 else wt[len(wt) // 2:]
            if last:
                _interleave(parts(conv, s, n)[:-1], wt + e1_tasks(n - 1))
                if n == NCT - 1:
                    for _, fn in e1_tasks(n):
                        fn()
            else:
                _interleave(parts(conv, s, n), wt)

        def tiles(s, n0, n1):
            for n in range(n0, n1):
                tile(s, n)

        def blk_a(s):
            if conv == 0:
                pl.when(flags[fl[0]] == 0)(functools.partial(tile, s, 0))
                pl.when(s != hi - 1)(functools.partial(tile, s, 1))
                pl.when(s == hi - 1)(functools.partial(tile, s, 1, True))
            else:
                pl.when(flags[fl[0]] == 0)(functools.partial(tiles, s, 0, 2))

        def blk_b(s):
            if conv == 0:
                pl.when(s != hi - 1)(functools.partial(tiles, s, 2, 4))
                pl.when(s == hi - 1)(functools.partial(tile, s, 2, True))
                pl.when(s + flags[fl[1]] == hi - 1)(functools.partial(tile, s, 3, True))
            else:
                pl.when(flags[fl[1]] == 0)(functools.partial(tiles, s, 2, 4))

        later = [(j, hf, next(groups)) for j in range(lo, hi) for hf in range(2)] if conv == 0 else []

        def start_later(s, hf):
            for j, hf_j, grp in later:
                if hf_j == hf:
                    pl.when(s == j)(functools.partial(w_start, *grp))

        def body(s, carry):
            w_wait(s, 1)
            start_later(s, 0)
            blk_a(s)
            if conv == 0:
                w_wait(s + 1, 0)
                start_later(s, 1)
            else:
                pl.when(s + 1 < NSTEP)(lambda: w_wait(jnp.minimum(s + 1, NSTEP - 1), 0))
            blk_b(s)
            return carry

        jax.lax.fori_loop(lo, hi, body, 0)

    conv_loop(0, 1, 4)

    start_next()
    assert next(groups, None) is None
    for cp in small_copies:
        cp.start()

    conv_loop(1, 4, NSTEP)

    for cp in small_copies:
        cp.wait()

    def proj():
        gev[...] = jnp.dot(gv[...], wsm[1], preferred_element_type=F32)
        for _, fn in e2_tasks(0):
            fn()
        for kt in range(NCT):
            _interleave([functools.partial(fe_part, kt)], e2_tasks(kt + 1) if kt + 1 < NCT else [])
        for _, fn in jtasks(0, 0):
            fn()
    block(proj)

    def jbody(a, carry):
        _interleave(jparts(0, a), jtasks(1, a))
        _interleave(jparts(1, a), jtasks(0, a + 1))
        return carry
    jax.lax.fori_loop(0, A - 1, jbody, 0)

    nt_last = T2 - NM * (A - 1)

    def jtail():
        _interleave(jparts(0, A - 1, nt_last), jtasks(1, A - 1, nt_last))
        for p in jparts(1, A - 1, nt_last):
            p()
    block(jtail)

    for b in range(B):
        for a in range(A):
            out_copy(b, a, NM if a + 1 < A else nt_last).wait()
    assert next(flag_ctr) <= NFLAGS


@jax.jit
def pallas_standalone__seq2seq_rnn_t_joint__speech_kernel(
    x: jax.Array,
    w1: jax.Array,
    w2: jax.Array,
    g: jax.Array,
    w_f: jax.Array,
    w_g: jax.Array,
    w_o: jax.Array,
):
    any_spec = pl.BlockSpec(memory_space=pl.ANY)
    out = pl.pallas_call(
        _kernel,
        out_shape=jax.ShapeDtypeStruct((B, T2 * U, D), BF16),
        in_specs=[pl.BlockSpec(memory_space=pltpu.SMEM)] + [any_spec] * 7,
        out_specs=any_spec,
        scratch_shapes=[
            pltpu.VMEM((NCT, B, T, LT), BF16),
            pltpu.VMEM((B, NCT, XROWS, LT), F32),
            [pltpu.VMEM((2, NC, R * (PV1 + 1), LT), BF16)] * NCT,
            [pltpu.VMEM((NC, M1, LT), F32)] * NCT,
            pltpu.VMEM((NSTEP, 8, D, D), BF16),
            [pltpu.VMEM((len(MULTI), LT, D), BF16)] * NCT,
            [pltpu.VMEM((len(MULTI), D, LT), BF16)] * NCT,
            pltpu.VMEM((Q2 + 2 * PAD, R, D), F32),
            [pltpu.VMEM((2, NC, R * (PV2 + 1), LT), BF16)] * NCT,
            pltpu.VMEM((NC, M2, D), F32),
            pltpu.VMEM((3, D, D), BF16),
            pltpu.VMEM((B * U, D), BF16),
            pltpu.VMEM((B * U, D), F32),
            [pltpu.VMEM((R * NM, LT), BF16)] * NCT,
            pltpu.VMEM((R * NM, D), F32),
            [pltpu.VMEM((U * NM, D), BF16)] * B,
            pltpu.VMEM((B, T2 * U, D), BF16),
            pltpu.SemaphoreType.DMA((NCT,)),
            pltpu.SemaphoreType.DMA((NCT + 2 * (NSTEP - 1),)),
            pltpu.SemaphoreType.DMA((4,)),
            pltpu.SemaphoreType.DMA((B * A,)),
        ],
        compiler_params=pltpu.CompilerParams(vmem_limit_bytes=120 * 1024 * 1024),
    )(jnp.zeros((NFLAGS,), jnp.int32), x, w1, w2, g.reshape(B * U, D), w_f, w_g, w_o)
    return out.reshape(B, T2, U, D)
```

```python
import functools
import itertools

import jax
import jax.numpy as jnp
import jax.experimental.pallas as pl
import jax.experimental.pallas.tpu as pltpu

F32 = jnp.float32
BF16 = jnp.bfloat16

B, T, D, K, U = 2, 1000, 512, 31, 8
PAD = K // 2
T1, T2 = T // 2, T // 4
A = 8
R = B * A
PV1, PV2 = 8, 4
Q1, Q2 = 16 * PV1, 16 * PV2
M1, M2 = R * PV1, R * PV2
XOFF = 16
XPITCH = Q1 + 1
XROWS = 1064
LT = 128
NCT = D // LT
HD = D // 2
NM = 8 * PV2
NSTEP = 8
NFLAGS = 32
S0_SPLIT = (9, 9, 9, 9)

COMBOS = list(itertools.product(range(3), repeat=3))
_WSET = {0: (0,), 1: (0, 1), 2: (1,)}
MULTI = [c for c in COMBOS if 1 in c]
MULTI_IDX = {c: i for i, c in enumerate(MULTI)}
CIDX = {c: i for i, c in enumerate(COMBOS)}
NC = len(COMBOS)


def _single_tap(c):
    return _WSET[c[0]][0] + 2 * _WSET[c[1]][0] + 4 * _WSET[c[2]][0]


def _cols(t):
    return slice(LT * t, LT * (t + 1))


def _half(hf):
    return slice(HD * hf, HD * (hf + 1))


def _gelu(x):
    c = 0.7978845608028654
    return 0.5 * x * (1.0 + jnp.tanh(c * (x + 0.044715 * (x * x * x))))


def _fir_in(seq, which=(0, 1, 2)):
    n = (len(seq) - 1) // 2
    out = {}
    if 0 in which:
        out[0] = [seq[2 * i] - seq[2 * i + 1] for i in range(n)]
    if 1 in which:
        out[1] = [seq[2 * i + 1] for i in range(n)]
    if 2 in which:
        out[2] = [seq[2 * i + 1] - seq[2 * i + 2] for i in range(n)]
    return out


def _output_transform(get_acc):
    p3 = {}
    for c1 in range(3):
        for c2 in range(3):
            m = get_acc((c1, c2, 1))
            p3[(c1, c2, 0)] = get_acc((c1, c2, 0)) + m
            p3[(c1, c2, 1)] = m - get_acc((c1, c2, 2))
    p2 = {}
    for c1 in range(3):
        for e3 in range(2):
            m = p3[(c1, 1, e3)]
            p2[(c1, 0, e3)] = p3[(c1, 0, e3)] + m
            p2[(c1, 1, e3)] = m - p3[(c1, 2, e3)]
    out = [None] * 8
    for e2 in range(2):
        for e3 in range(2):
            m = p2[(1, e2, e3)]
            out[0 + 2 * e2 + 4 * e3] = p2[(0, e2, e3)] + m
            out[1 + 2 * e2 + 4 * e3] = m - p2[(2, e2, e3)]
    return out


def _tap(s, d):
    return 16 * ((s % 4) // 2) + 2 * d + s % 2


def _interleave(parts, tasks):
    total = sum(c for c, _ in tasks) or 1
    n, done, ti = len(parts), 0, 0
    for i, part in enumerate(parts):
        part()
        while ti < len(tasks) and done * n < total * (i + 1) - (total if i + 1 < n else 0) * 0.5:
            done += tasks[ti][0]
            tasks[ti][1]()
            ti += 1
    for _, fn in tasks[ti:]:
        fn()


WR = 8


def _kernel(x_hbm, w1_hbm, w2_hbm, g_hbm, wf_hbm, wg_hbm, wo_hbm, out_hbm,
            xb, xf, d1, acc1, wraw, vt0, vth, hs, d2, acc2, wsm, gv, gev, fb, fe, jb, ov,
            flags, sem_x, sem_w, sem_s, sem_o):
    w_hbm = (w1_hbm, w2_hbm)
    flag_ctr = itertools.count()
    for i in range(NFLAGS):
        flags[i] = 0

    def block(fn):
        pl.when(flags[next(flag_ctr)] == 0)(fn)

    def x_copies(ct):
        return [pltpu.make_async_copy(x_hbm.at[:, :, _cols(ct)], xb.at[ct], sem_x.at[ct])]

    def w0_copies(kt):
        return [pltpu.make_async_copy(w1_hbm.at[_tap(0, d), _cols(kt), :],
                                      wraw.at[0, d, _cols(kt), :], sem_w.at[kt])
                for d in range(8)]

    def w_sem(s, hf):
        return sem_w.at[NCT + 2 * (s - 1) + hf]

    def w_start(s, hf):
        for d in range(8):
            if _tap(s, d) < K:
                pltpu.make_async_copy(w_hbm[s // 4].at[_tap(s, d), :, _half(hf)],
                                      wraw.at[s, d, :, _half(hf)], w_sem(s, hf)).start()

    def w_wait(s, hf):
        def one(d):
            pltpu.make_async_copy(w1_hbm.at[0, :, _half(hf)],
                                  wraw.at[s, d, :, _half(hf)], w_sem(s, hf)).wait()
        for d in range(7):
            one(d)
        if isinstance(s, int):
            if _tap(s, 7) < K:
                one(7)
        else:
            pl.when(s % 4 != 3)(functools.partial(one, 7))

    small_copies = [
        pltpu.make_async_copy(g_hbm, gv, sem_s.at[0]),
        pltpu.make_async_copy(wg_hbm, wsm.at[1], sem_s.at[1]),
        pltpu.make_async_copy(wf_hbm, wsm.at[0], sem_s.at[2]),
        pltpu.make_async_copy(wo_hbm, wsm.at[2], sem_s.at[3]),
    ]

    def wsums(d):
        lv = {}
        for b2 in range(2):
            for b1 in range(2):
                lo, hi = d[4 * b2 + 2 * b1], d[4 * b2 + 2 * b1 + 1]
                lv[(0, b1, b2)], lv[(1, b1, b2)], lv[(2, b1, b2)] = lo, lo + hi, hi
        lw = {}
        for b2 in range(2):
            for c1 in range(3):
                lo, hi = lv[(c1, 0, b2)], lv[(c1, 1, b2)]
                lw[(c1, 0, b2)], lw[(c1, 1, b2)], lw[(c1, 2, b2)] = lo, lo + hi, hi
        for c1 in range(3):
            for c2 in range(3):
                lo, hi = lw[(c1, c2, 0)], lw[(c1, c2, 1)]
                for c3, v in ((0, lo), (1, lo + hi), (2, hi)):
                    if (c1, c2, c3) in MULTI_IDX:
                        yield (c1, c2, c3), v

    def wchunk0(kt, r0, hf):
        rs = slice(LT * kt + r0, LT * kt + r0 + WR)
        for c, v in wsums([wraw[0, i, rs, _half(hf)].astype(F32) for i in range(8)]):
            vt0[kt][MULTI_IDX[c], r0:r0 + WR, _half(hf)] = v.astype(BF16)

    def wchunk(s, r0, n):
        rs = slice(r0, r0 + 2 * WR)
        for c, v in wsums([wraw[s, i, rs, _cols(n)].astype(F32) for i in range(8)]):
            vth[n][MULTI_IDX[c], rs, :] = v.astype(BF16)

    def w0_tasks(kt):
        return [(19, functools.partial(wchunk0, kt, r0, hf))
                for r0 in range(0, LT, WR) for hf in range(2)]

    def wh_tasks(s, hf):
        return [(19, functools.partial(wchunk, s, r0, n))
                for r0 in range(0, D, 2 * WR) for n in (2 * hf, 2 * hf + 1)]

    def in_win(get_y, d_ref, h, ct, r, c1):
        y = [get_y(8 * r + o) if (c1 != 1 or o % 2 == 1) and (c1, o) not in ((0, 14), (2, 0)) else None
             for o in range(15)]
        l1 = _fir_in(y, (c1,))[c1]
        l2 = _fir_in(l1)
        for c2 in range(3):
            l3 = _fir_in(l2[c2])
            for c3 in range(3):
                d_ref[ct][h, CIDX[(c1, c2, c3)], R * r:R * (r + 1), :] = l3[c3][0].astype(BF16)

    def in_tasks(get_y, d_ref, pv, h, ct):
        return [(16, functools.partial(in_win, get_y, d_ref, h, ct, r, c1))
                for r in range(pv + 1) for c1 in range(3)]

    def y1(h, ct):
        def get(i):
            m = 2 * i - PAD + h
            st = XOFF + m + (m // Q1) * (XPITCH - Q1)
            return jnp.concatenate(
                [xf[b, ct, pl.ds(st, A, stride=XPITCH), :] for b in range(B)], axis=0)
        return get

    def y2(h, ct):
        return lambda i: hs[2 * i + h, :, _cols(ct)]

    def xconv(b, ct, a):
        n = min(Q1, T - Q1 * a)
        xf[b, ct, XOFF + XPITCH * a:XOFF + XPITCH * a + n, :] = xb[ct, b, Q1 * a:Q1 * a + n, :].astype(F32)

    def xtasks(ct):
        out = [(16, functools.partial(xconv, b, ct, a)) for b in range(B) for a in range(A)]
        return out + in_tasks(y1(0, ct), d1, PV1, 0, ct)

    def x1tasks(ct):
        return in_tasks(y1(1, ct), d1, PV1, 1, ct)

    def e1a(n, r, b):
        outs = _output_transform(lambda c: acc1[n][CIDX[c], R * r + A * b:R * r + A * (b + 1), :])
        for e in range(8):
            hs[PAD + 8 * r + e, A * b:A * (b + 1), _cols(n)] = outs[e]

    def e1b(n, r, b):
        a_idx = jax.lax.broadcasted_iota(jnp.int32, (A, LT), 0)
        rows = slice(A * b, A * (b + 1))
        for e in range(8):
            m = 8 * r + e
            v = _gelu(hs[PAD + m, rows, _cols(n)])
            if Q2 * (A - 1) + m >= T1:
                v = jnp.where(a_idx == A - 1, 0.0, v)
            hs[PAD + m, rows, _cols(n)] = v
            if m < PAD:
                hs[PAD + Q2 + m, rows, _cols(n)] = jnp.where(a_idx == A - 1, 0.0, pltpu.roll(v, A - 1, 0))
            if m >= Q2 - PAD:
                hs[PAD + m - Q2, rows, _cols(n)] = jnp.where(a_idx == 0, 0.0, pltpu.roll(v, 1, 0))

    def e1_tasks(n, lag=3):
        units = [(r, b) for r in range(PV1) for b in range(B)]
        out = []
        for i in range(len(units) + lag):
            if i < len(units):
                out.append((14, functools.partial(e1a, n, *units[i])))
            if i >= lag:
                out.append((26, functools.partial(e1b, n, *units[i - lag])))
        for h in range(2):
            out += in_tasks(y2(h, n), d2, PV2, h, n)
        return out

    def e2(n, r):
        outs = _output_transform(lambda c: acc2[CIDX[c], R * r:R * (r + 1), _cols(n)])
        for e in range(8):
            m = 8 * r + e
            fb[n][R * m:R * (m + 1), :] = _gelu(outs[e]).astype(BF16)

    def e2_tasks(n):
        return [(70, functools.partial(e2, n, r)) for r in range(PV2)]

    def part0(c, kt):
        if c in MULTI_IDX:
            w = vt0[kt][MULTI_IDX[c]]
        else:
            w = wraw[0, _single_tap(c), _cols(kt), :]
        p = jnp.dot(d1[kt][0, CIDX[c], 0:M1, :], w, preferred_element_type=F32)
        for n in range(NCT):
            if kt == 0:
                acc1[n][CIDX[c]] = p[:, _cols(n)]
            else:
                acc1[n][CIDX[c]] += p[:, _cols(n)]

    def part(conv, s, c, n):
        d_ref, m_rows = ((d1, M1), (d2, M2))[conv]
        if c in MULTI_IDX:
            w = vth[n][MULTI_IDX[c]]
        else:
            w = wraw[s, _single_tap(c), :, _cols(n)]
        r0 = pl.multiple_of(((s % 4) // 2) * R, R)
        lhs = jnp.concatenate([d_ref[ct][s % 2, CIDX[c], pl.ds(r0, m_rows), :] for ct in range(NCT)], axis=1)
        p = jnp.dot(lhs, w, preferred_element_type=F32)
        if conv == 0:
            acc1[n][CIDX[c]] += p
        else:
            acc2[CIDX[c], :, _cols(n)] += p

    def parts(conv, s, n):
        return [functools.partial(part, conv, s, c, n) for c in COMBOS]

    def jbuild(b, a, m0):
        geb = gev[U * b:U * (b + 1), :]
        js = []
        for m in range(m0, m0 + 2):
            frow = fe[pl.ds(R * m + A * b + a, 1), :]
            js.append(jnp.tanh(jnp.broadcast_to(frow, (U, D)) + geb))
        jb[b][U * m0:U * (m0 + 2), :] = jnp.concatenate(js, axis=0).astype(BF16)

    def jtasks(b, a, nt=NM):
        return [(8, functools.partial(jbuild, b, a, m0)) for m0 in range(0, nt, 2)]

    def out_copy(b, a, nt):
        r0 = U * NM * a if isinstance(a, int) else pl.multiple_of(U * NM * a, U * NM)
        rows = pl.ds(r0, U * nt)
        return pltpu.make_async_copy(ov.at[b, rows, :], out_hbm.at[b, rows, :], sem_o.at[A * b + a])

    def jpart(b, a, nt, n):
        r0 = U * NM * a if isinstance(a, int) else pl.multiple_of(U * NM * a, U * NM)
        o = jnp.dot(jb[b][0:U * nt, :], wsm[2, :, _cols(n)], preferred_element_type=F32)
        ov[b, pl.ds(r0, U * nt), _cols(n)] = o.astype(BF16)
        if n == NCT - 1:
            out_copy(b, a, nt).start()

    def jparts(b, a, nt=NM):
        return [functools.partial(jpart, b, a, nt, n) for n in range(NCT)]

    def fe_part(kt):
        p = jnp.dot(fb[kt][...], wsm[0, _cols(kt), :], preferred_element_type=F32)
        if kt == 0:
            fe[...] = p
        else:
            fe[...] += p

    groups = iter([(s, hf) for s in range(1, NSTEP) for hf in range(2)])

    def start_next():
        w_start(*next(groups))

    for cp in x_copies(0) + w0_copies(0):
        cp.start()

    def init():
        tail0 = XOFF + XPITCH * (A - 1) + T - Q1 * (A - 1)
        for b in range(B):
            for ct in range(NCT):
                xf[b, ct, 0:XOFF, :] = jnp.zeros((XOFF, LT), F32)
                xf[b, ct, tail0:XROWS, :] = jnp.zeros((XROWS - tail0, LT), F32)
        for s in (3, 7):
            wraw[s, 7] = jnp.zeros((D, D), BF16)
        acc2[...] = jnp.zeros(acc2.shape, F32)
    block(init)
    for cp in x_copies(1) + w0_copies(1):
        cp.start()

    for cp in x_copies(0):
        cp.wait()

    def prep0():
        for _, fn in xtasks(0):
            fn()
    block(prep0)
    for cp in w0_copies(0):
        cp.wait()
    for cp in x_copies(2) + w0_copies(2):
        cp.start()

    for kt in range(NCT):
        order = [c for c in COMBOS if c not in MULTI_IDX] + MULTI if kt == 0 else COMBOS
        p0 = [functools.partial(part0, c, kt) for c in order]
        sp = S0_SPLIT[kt]
        if kt == 0:
            block(lambda p0=p0, sp=sp: (_interleave(p0[:NC - len(MULTI)], w0_tasks(0)),
                                        _interleave(p0[NC - len(MULTI):sp], [])) and None)
        else:
            block(functools.partial(_interleave, p0[:sp], x1tasks(kt - 1)))
        if kt + 1 < NCT:
            for cp in x_copies(kt + 1) + w0_copies(kt + 1):
                cp.wait()
            if kt == 0:
                for cp in x_copies(3) + w0_copies(3):
                    cp.start()
            else:
                start_next()
            if kt == 2:
                start_next()
            tasks = xtasks(kt + 1) + w0_tasks(kt + 1)
        else:
            w_wait(1, 0)
            for _ in range(4):
                start_next()
            tasks = wh_tasks(1, 0) + x1tasks(NCT - 1)
        block(functools.partial(_interleave, p0[sp:], tasks))

    def conv_loop(conv, lo, hi):
        fl = [next(flag_ctr) for _ in range(2)]

        def tile(s, n, last=False):
            wt = wh_tasks(s, 1) if n < 2 else wh_tasks(jnp.minimum(s + 1, NSTEP - 1), 0)
            wt = wt[:len(wt) // 2] if n % 2 == 0 else wt[len(wt) // 2:]
            if last:
                _interleave(parts(conv, s, n)[:-1], wt + e1_tasks(n - 1))
                if n == NCT - 1:
                    for _, fn in e1_tasks(n):
                        fn()
            else:
                _interleave(parts(conv, s, n), wt)

        def tiles(s, n0, n1):
            for n in range(n0, n1):
                tile(s, n)

        def blk_a(s):
            if conv == 0:
                pl.when(flags[fl[0]] == 0)(functools.partial(tile, s, 0))
                pl.when(s != hi - 1)(functools.partial(tile, s, 1))
                pl.when(s == hi - 1)(functools.partial(tile, s, 1, True))
            else:
                pl.when(flags[fl[0]] == 0)(functools.partial(tiles, s, 0, 2))

        def blk_b(s):
            if conv == 0:
                pl.when(s != hi - 1)(functools.partial(tiles, s, 2, 4))
                pl.when(s == hi - 1)(functools.partial(tile, s, 2, True))
                pl.when(s + flags[fl[1]] == hi - 1)(functools.partial(tile, s, 3, True))
            else:
                pl.when(flags[fl[1]] == 0)(functools.partial(tiles, s, 2, 4))

        later = [(j, hf, next(groups)) for j in range(lo, hi) for hf in range(2)] if conv == 0 else []

        def start_later(s, hf):
            for j, hf_j, grp in later:
                if hf_j == hf:
                    pl.when(s == j)(functools.partial(w_start, *grp))

        def body(s, carry):
            w_wait(s, 1)
            start_later(s, 0)
            blk_a(s)
            if conv == 0:
                w_wait(s + 1, 0)
                start_later(s, 1)
            else:
                pl.when(s + 1 < NSTEP)(lambda: w_wait(jnp.minimum(s + 1, NSTEP - 1), 0))
            blk_b(s)
            return carry

        jax.lax.fori_loop(lo, hi, body, 0)

    conv_loop(0, 1, 4)

    start_next()
    assert next(groups, None) is None
    for cp in small_copies:
        cp.start()

    conv_loop(1, 4, NSTEP)

    for cp in small_copies:
        cp.wait()

    def proj():
        gev[...] = jnp.dot(gv[...], wsm[1], preferred_element_type=F32)
        for _, fn in e2_tasks(0):
            fn()
        for kt in range(NCT):
            _interleave([functools.partial(fe_part, kt)], e2_tasks(kt + 1) if kt + 1 < NCT else [])
        for _, fn in jtasks(0, 0):
            fn()
    block(proj)

    def jbody(a, carry):
        _interleave(jparts(0, a), jtasks(1, a))
        _interleave(jparts(1, a), jtasks(0, a + 1))
        return carry
    jax.lax.fori_loop(0, A - 1, jbody, 0)

    nt_last = T2 - NM * (A - 1)

    def jtail():
        _interleave(jparts(0, A - 1, nt_last), jtasks(1, A - 1, nt_last))
        for p in jparts(1, A - 1, nt_last):
            p()
    block(jtail)

    for b in range(B):
        for a in range(A):
            out_copy(b, a, NM if a + 1 < A else nt_last).wait()
    assert next(flag_ctr) <= NFLAGS


@jax.jit
def pallas_standalone__seq2seq_rnn_t_joint__speech_kernel(
    x: jax.Array,
    w1: jax.Array,
    w2: jax.Array,
    g: jax.Array,
    w_f: jax.Array,
    w_g: jax.Array,
    w_o: jax.Array,
):
    any_spec = pl.BlockSpec(memory_space=pl.ANY)
    out = pl.pallas_call(
        _kernel,
        out_shape=jax.ShapeDtypeStruct((B, T2 * U, D), BF16),
        in_specs=[any_spec] * 7,
        out_specs=any_spec,
        scratch_shapes=[
            pltpu.VMEM((NCT, B, T, LT), BF16),
            pltpu.VMEM((B, NCT, XROWS, LT), F32),
            [pltpu.VMEM((2, NC, R * (PV1 + 4), LT), BF16)] * NCT,
            [pltpu.VMEM((NC, M1, LT), F32)] * NCT,
            pltpu.VMEM((NSTEP, 8, D, D), BF16),
            [pltpu.VMEM((len(MULTI), LT, D), BF16)] * NCT,
            [pltpu.VMEM((len(MULTI), D, LT), BF16)] * NCT,
            pltpu.VMEM((Q2 + 2 * PAD, R, D), F32),
            [pltpu.VMEM((2, NC, R * (PV2 + 4), LT), BF16)] * NCT,
            pltpu.VMEM((NC, M2, D), F32),
            pltpu.VMEM((3, D, D), BF16),
            pltpu.VMEM((B * U, D), BF16),
            pltpu.VMEM((B * U, D), F32),
            [pltpu.VMEM((R * NM, LT), BF16)] * NCT,
            pltpu.VMEM((R * NM, D), F32),
            [pltpu.VMEM((U * NM, D), BF16)] * B,
            pltpu.VMEM((B, T2 * U, D), BF16),
            pltpu.SMEM((NFLAGS,), jnp.int32),
            pltpu.SemaphoreType.DMA((NCT,)),
            pltpu.SemaphoreType.DMA((NCT + 2 * (NSTEP - 1),)),
            pltpu.SemaphoreType.DMA((4,)),
            pltpu.SemaphoreType.DMA((B * A,)),
        ],
        compiler_params=pltpu.CompilerParams(vmem_limit_bytes=120 * 1024 * 1024),
    )(x, w1, w2, g.reshape(B * U, D), w_f, w_g, w_o)
    return out.reshape(B, T2, U, D)
```

```python
import functools
import itertools

import jax
import jax.numpy as jnp
import jax.experimental.pallas as pl
import jax.experimental.pallas.tpu as pltpu

F32 = jnp.float32
BF16 = jnp.bfloat16

B, T, D, K, U = 2, 1000, 512, 31, 8
PAD = K // 2
T1, T2 = T // 2, T // 4
A = 8
R = B * A
PV1, PV2 = 8, 4
Q1, Q2 = 16 * PV1, 16 * PV2
M1, M2 = R * PV1, R * PV2
XOFF = 16
XPITCH = Q1 + 1
XROWS = 1064
LT = 128
NCT = D // LT
HD = D // 2
NM = 8 * PV2
NSTEP = 8
NFLAGS = 32
S0_SPLIT = (9, 9, 9, 9)

COMBOS = list(itertools.product(range(3), repeat=3))
_WSET = {0: (0,), 1: (0, 1), 2: (1,)}
MULTI = [c for c in COMBOS if 1 in c]
MULTI_IDX = {c: i for i, c in enumerate(MULTI)}
CIDX = {c: i for i, c in enumerate(COMBOS)}
NC = len(COMBOS)


def _single_tap(c):
    return _WSET[c[0]][0] + 2 * _WSET[c[1]][0] + 4 * _WSET[c[2]][0]


def _cols(t):
    return slice(LT * t, LT * (t + 1))


def _half(hf):
    return slice(HD * hf, HD * (hf + 1))


def _gelu(x):
    c = 0.7978845608028654
    return 0.5 * x * (1.0 + jnp.tanh(c * (x + 0.044715 * (x * x * x))))


def _fir_in(seq, which=(0, 1, 2)):
    n = (len(seq) - 1) // 2
    out = {}
    if 0 in which:
        out[0] = [seq[2 * i] - seq[2 * i + 1] for i in range(n)]
    if 1 in which:
        out[1] = [seq[2 * i + 1] for i in range(n)]
    if 2 in which:
        out[2] = [seq[2 * i + 1] - seq[2 * i + 2] for i in range(n)]
    return out


def _output_transform(get_acc):
    p3 = {}
    for c1 in range(3):
        for c2 in range(3):
            m = get_acc((c1, c2, 1))
            p3[(c1, c2, 0)] = get_acc((c1, c2, 0)) + m
            p3[(c1, c2, 1)] = m - get_acc((c1, c2, 2))
    p2 = {}
    for c1 in range(3):
        for e3 in range(2):
            m = p3[(c1, 1, e3)]
            p2[(c1, 0, e3)] = p3[(c1, 0, e3)] + m
            p2[(c1, 1, e3)] = m - p3[(c1, 2, e3)]
    out = [None] * 8
    for e2 in range(2):
        for e3 in range(2):
            m = p2[(1, e2, e3)]
            out[0 + 2 * e2 + 4 * e3] = p2[(0, e2, e3)] + m
            out[1 + 2 * e2 + 4 * e3] = m - p2[(2, e2, e3)]
    return out


def _tap(s, d):
    return 16 * ((s % 4) // 2) + 2 * d + s % 2


def _interleave(parts, tasks):
    total = sum(c for c, _ in tasks) or 1
    n, done, ti = len(parts), 0, 0
    for i, part in enumerate(parts):
        part()
        while ti < len(tasks) and done * n < total * (i + 1) - (total if i + 1 < n else 0) * 0.5:
            done += tasks[ti][0]
            tasks[ti][1]()
            ti += 1
    for _, fn in tasks[ti:]:
        fn()


WR = 8


def _kernel(x_hbm, w1_hbm, w2_hbm, g_hbm, wf_hbm, wg_hbm, wo_hbm, out_hbm,
            xb, xf, d1, acc1, wraw, vt0, vth, hs, d2, acc2, wsm, gv, gev, fb, fe, jb, ov,
            flags, sem_x, sem_w, sem_s, sem_o):
    w_hbm = (w1_hbm, w2_hbm)
    flag_ctr = itertools.count()
    for i in range(NFLAGS):
        flags[i] = 0

    def block(fn):
        pl.when(flags[next(flag_ctr)] == 0)(fn)

    def x_copies(ct):
        return [pltpu.make_async_copy(x_hbm.at[:, :, _cols(ct)], xb.at[ct], sem_x.at[ct])]

    def w0_copies(kt):
        return [pltpu.make_async_copy(w1_hbm.at[_tap(0, d), _cols(kt), :],
                                      wraw.at[0, d, _cols(kt), :], sem_w.at[kt])
                for d in range(8)]

    def w_sem(s, hf):
        return sem_w.at[NCT + 2 * (s - 1) + hf]

    def w_start(s, hf):
        for d in range(8):
            if _tap(s, d) < K:
                pltpu.make_async_copy(w_hbm[s // 4].at[_tap(s, d), :, _half(hf)],
                                      wraw.at[s, d, :, _half(hf)], w_sem(s, hf)).start()

    def w_wait(s, hf):
        def one(d):
            pltpu.make_async_copy(w1_hbm.at[0, :, _half(hf)],
                                  wraw.at[s, d, :, _half(hf)], w_sem(s, hf)).wait()
        for d in range(7):
            one(d)
        if isinstance(s, int):
            if _tap(s, 7) < K:
                one(7)
        else:
            pl.when(s % 4 != 3)(functools.partial(one, 7))

    small_copies = [
        pltpu.make_async_copy(g_hbm, gv, sem_s.at[0]),
        pltpu.make_async_copy(wg_hbm, wsm.at[1], sem_s.at[1]),
        pltpu.make_async_copy(wf_hbm, wsm.at[0], sem_s.at[2]),
        pltpu.make_async_copy(wo_hbm, wsm.at[2], sem_s.at[3]),
    ]

    def wsums(d):
        lv = {}
        for b2 in range(2):
            for b1 in range(2):
                lo, hi = d[4 * b2 + 2 * b1], d[4 * b2 + 2 * b1 + 1]
                lv[(0, b1, b2)], lv[(1, b1, b2)], lv[(2, b1, b2)] = lo, lo + hi, hi
        lw = {}
        for b2 in range(2):
            for c1 in range(3):
                lo, hi = lv[(c1, 0, b2)], lv[(c1, 1, b2)]
                lw[(c1, 0, b2)], lw[(c1, 1, b2)], lw[(c1, 2, b2)] = lo, lo + hi, hi
        for c1 in range(3):
            for c2 in range(3):
                lo, hi = lw[(c1, c2, 0)], lw[(c1, c2, 1)]
                for c3, v in ((0, lo), (1, lo + hi), (2, hi)):
                    if (c1, c2, c3) in MULTI_IDX:
                        yield (c1, c2, c3), v

    def wchunk0(kt, r0, hf):
        rs = slice(LT * kt + r0, LT * kt + r0 + WR)
        for c, v in wsums([wraw[0, i, rs, _half(hf)].astype(F32) for i in range(8)]):
            vt0[kt][MULTI_IDX[c], r0:r0 + WR, _half(hf)] = v.astype(BF16)

    def wchunk(s, r0, n):
        rs = slice(r0, r0 + 2 * WR)
        for c, v in wsums([wraw[s, i, rs, _cols(n)].astype(F32) for i in range(8)]):
            vth[n][MULTI_IDX[c], rs, :] = v.astype(BF16)

    def w0_tasks(kt):
        return [(19, functools.partial(wchunk0, kt, r0, hf))
                for r0 in range(0, LT, WR) for hf in range(2)]

    def wh_tasks(s, hf):
        return [(19, functools.partial(wchunk, s, r0, n))
                for r0 in range(0, D, 2 * WR) for n in (2 * hf, 2 * hf + 1)]

    def in_win(get_y, d_ref, h, ct, r, c1):
        y = [get_y(8 * r + o) if (c1 != 1 or o % 2 == 1) and (c1, o) not in ((0, 14), (2, 0)) else None
             for o in range(15)]
        l1 = _fir_in(y, (c1,))[c1]
        l2 = _fir_in(l1)
        for c2 in range(3):
            l3 = _fir_in(l2[c2])
            for c3 in range(3):
                d_ref[ct][h, CIDX[(c1, c2, c3)], R * r:R * (r + 1), :] = l3[c3][0].astype(BF16)

    def in_tasks(get_y, d_ref, pv, h, ct):
        return [(16, functools.partial(in_win, get_y, d_ref, h, ct, r, c1))
                for r in range(pv + 1) for c1 in range(3)]

    def y1(h, ct):
        def get(i):
            m = 2 * i - PAD + h
            st = XOFF + m + (m // Q1) * (XPITCH - Q1)
            return jnp.concatenate(
                [xf[b, ct, pl.ds(st, A, stride=XPITCH), :] for b in range(B)], axis=0)
        return get

    def y2(h, ct):
        return lambda i: hs[2 * i + h, :, _cols(ct)]

    def xconv(b, ct, a):
        n = min(Q1, T - Q1 * a)
        xf[b, ct, XOFF + XPITCH * a:XOFF + XPITCH * a + n, :] = xb[ct, b, Q1 * a:Q1 * a + n, :].astype(F32)

    def xtasks(ct):
        out = [(16, functools.partial(xconv, b, ct, a)) for b in range(B) for a in range(A)]
        return out + in_tasks(y1(0, ct), d1, PV1, 0, ct)

    def x1tasks(ct):
        return in_tasks(y1(1, ct), d1, PV1, 1, ct)

    def e1a(n, r, b):
        outs = _output_transform(lambda c: acc1[n][CIDX[c], R * r + A * b:R * r + A * (b + 1), :])
        for e in range(8):
            hs[PAD + 8 * r + e, A * b:A * (b + 1), _cols(n)] = outs[e]

    def e1b(n, r, b):
        a_idx = jax.lax.broadcasted_iota(jnp.int32, (A, LT), 0)
        rows = slice(A * b, A * (b + 1))
        for e in range(8):
            m = 8 * r + e
            v = _gelu(hs[PAD + m, rows, _cols(n)])
            if Q2 * (A - 1) + m >= T1:
                v = jnp.where(a_idx == A - 1, 0.0, v)
            hs[PAD + m, rows, _cols(n)] = v
            if m < PAD:
                hs[PAD + Q2 + m, rows, _cols(n)] = jnp.where(a_idx == A - 1, 0.0, pltpu.roll(v, A - 1, 0))
            if m >= Q2 - PAD:
                hs[PAD + m - Q2, rows, _cols(n)] = jnp.where(a_idx == 0, 0.0, pltpu.roll(v, 1, 0))

    def e1_tasks(n, lag=3):
        units = [(r, b) for r in range(PV1) for b in range(B)]
        out = []
        for i in range(len(units) + lag):
            if i < len(units):
                out.append((14, functools.partial(e1a, n, *units[i])))
            if i >= lag:
                out.append((26, functools.partial(e1b, n, *units[i - lag])))
        for h in range(2):
            out += in_tasks(y2(h, n), d2, PV2, h, n)
        return out

    def e2(n, r):
        outs = _output_transform(lambda c: acc2[CIDX[c], R * r:R * (r + 1), _cols(n)])
        for e in range(8):
            m = 8 * r + e
            fb[n][R * m:R * (m + 1), :] = _gelu(outs[e]).astype(BF16)

    def e2_tasks(n):
        return [(70, functools.partial(e2, n, r)) for r in range(PV2)]

    def part0(c, kt):
        if c in MULTI_IDX:
            w = vt0[kt][MULTI_IDX[c]]
        else:
            w = wraw[0, _single_tap(c), _cols(kt), :]
        p = jnp.dot(d1[kt][0, CIDX[c], 0:M1, :], w, preferred_element_type=F32)
        for n in range(NCT):
            if kt == 0:
                acc1[n][CIDX[c]] = p[:, _cols(n)]
            else:
                acc1[n][CIDX[c]] += p[:, _cols(n)]

    def part(conv, st, c, n):
        s, h, r0 = st
        d_ref, m_rows = ((d1, M1), (d2, M2))[conv]
        if c in MULTI_IDX:
            w = vth[n][MULTI_IDX[c]]
        else:
            w = wraw[s, _single_tap(c), :, _cols(n)]
        lhs = jnp.concatenate([d_ref[ct][h, CIDX[c], pl.ds(r0, m_rows), :] for ct in range(NCT)], axis=1)
        p = jnp.dot(lhs, w, preferred_element_type=F32)
        if conv == 0:
            acc1[n][CIDX[c]] += p
        else:
            acc2[CIDX[c], :, _cols(n)] += p

    def parts(conv, st, n):
        return [functools.partial(part, conv, st, c, n) for c in COMBOS]

    def jbuild(b, a, m0):
        geb = gev[U * b:U * (b + 1), :]
        js = []
        for m in range(m0, m0 + 2):
            frow = fe[pl.ds(R * m + A * b + a, 1), :]
            js.append(jnp.tanh(jnp.broadcast_to(frow, (U, D)) + geb))
        jb[b][U * m0:U * (m0 + 2), :] = jnp.concatenate(js, axis=0).astype(BF16)

    def jtasks(b, a, nt=NM):
        return [(8, functools.partial(jbuild, b, a, m0)) for m0 in range(0, nt, 2)]

    def out_copy(b, a, nt):
        r0 = U * NM * a if isinstance(a, int) else pl.multiple_of(U * NM * a, U * NM)
        rows = pl.ds(r0, U * nt)
        return pltpu.make_async_copy(ov.at[b, rows, :], out_hbm.at[b, rows, :], sem_o.at[A * b + a])

    def jpart(b, a, nt, n):
        r0 = U * NM * a if isinstance(a, int) else pl.multiple_of(U * NM * a, U * NM)
        o = jnp.dot(jb[b][0:U * nt, :], wsm[2, :, _cols(n)], preferred_element_type=F32)
        ov[b, pl.ds(r0, U * nt), _cols(n)] = o.astype(BF16)
        if n == NCT - 1:
            out_copy(b, a, nt).start()

    def jparts(b, a, nt=NM):
        return [functools.partial(jpart, b, a, nt, n) for n in range(NCT)]

    def fe_part(kt):
        p = jnp.dot(fb[kt][...], wsm[0, _cols(kt), :], preferred_element_type=F32)
        if kt == 0:
            fe[...] = p
        else:
            fe[...] += p

    groups = iter([(s, hf) for s in range(1, NSTEP) for hf in range(2)])

    def start_next():
        w_start(*next(groups))

    for cp in x_copies(0) + w0_copies(0):
        cp.start()

    def init():
        tail0 = XOFF + XPITCH * (A - 1) + T - Q1 * (A - 1)
        for b in range(B):
            for ct in range(NCT):
                xf[b, ct, 0:XOFF, :] = jnp.zeros((XOFF, LT), F32)
                xf[b, ct, tail0:XROWS, :] = jnp.zeros((XROWS - tail0, LT), F32)
        for s in (3, 7):
            wraw[s, 7] = jnp.zeros((D, D), BF16)
        acc2[...] = jnp.zeros(acc2.shape, F32)
    block(init)
    for cp in x_copies(1) + w0_copies(1):
        cp.start()

    for cp in x_copies(0):
        cp.wait()

    def prep0():
        for _, fn in xtasks(0):
            fn()
    block(prep0)
    for cp in w0_copies(0):
        cp.wait()
    for cp in x_copies(2) + w0_copies(2):
        cp.start()

    for kt in range(NCT):
        order = [c for c in COMBOS if c not in MULTI_IDX] + MULTI if kt == 0 else COMBOS
        p0 = [functools.partial(part0, c, kt) for c in order]
        sp = S0_SPLIT[kt]
        if kt == 0:
            block(lambda p0=p0, sp=sp: (_interleave(p0[:NC - len(MULTI)], w0_tasks(0)),
                                        _interleave(p0[NC - len(MULTI):sp], [])) and None)
        else:
            block(functools.partial(_interleave, p0[:sp], x1tasks(kt - 1)))
        if kt + 1 < NCT:
            for cp in x_copies(kt + 1) + w0_copies(kt + 1):
                cp.wait()
            if kt == 0:
                for cp in x_copies(3) + w0_copies(3):
                    cp.start()
            else:
                start_next()
            if kt == 2:
                start_next()
            tasks = xtasks(kt + 1) + w0_tasks(kt + 1)
        else:
            w_wait(1, 0)
            for _ in range(4):
                start_next()
            tasks = wh_tasks(1, 0) + x1tasks(NCT - 1)
        block(functools.partial(_interleave, p0[sp:], tasks))

    def conv_loop(conv, lo, hi):
        fl = [next(flag_ctr) for _ in range(2)]

        def tile(st, nxt, n, last=False):
            wt = wh_tasks(st[0], 1) if n < 2 else wh_tasks(nxt, 0)
            wt = wt[:len(wt) // 2] if n % 2 == 0 else wt[len(wt) // 2:]
            if last:
                _interleave(parts(conv, st, n)[:-1], wt + e1_tasks(n - 1))
                if n == NCT - 1:
                    for _, fn in e1_tasks(n):
                        fn()
            else:
                _interleave(parts(conv, st, n), wt)

        def tiles(st, nxt, n0, n1):
            for n in range(n0, n1):
                tile(st, nxt, n)

        def blk_a(st, nxt):
            s = st[0]
            if conv == 0:
                pl.when(flags[fl[0]] == 0)(functools.partial(tile, st, nxt, 0))
                pl.when(s != hi - 1)(functools.partial(tile, st, nxt, 1))
                pl.when(s == hi - 1)(functools.partial(tile, st, nxt, 1, True))
            else:
                pl.when(flags[fl[0]] == 0)(functools.partial(tiles, st, nxt, 0, 2))

        def blk_b(st, nxt):
            s = st[0]
            if conv == 0:
                pl.when(s != hi - 1)(functools.partial(tiles, st, nxt, 2, 4))
                pl.when(s == hi - 1)(functools.partial(tile, st, nxt, 2, True))
                pl.when(s + flags[fl[1]] == hi - 1)(functools.partial(tile, st, nxt, 3, True))
            else:
                pl.when(flags[fl[1]] == 0)(functools.partial(tiles, st, nxt, 2, 4))

        later = [(j, hf, next(groups)) for j in range(lo, hi) for hf in range(2)] if conv == 0 else []

        def start_later(s, hf):
            for j, hf_j, grp in later:
                if hf_j == hf:
                    pl.when(s == j)(functools.partial(w_start, *grp))

        def body(s, carry):
            st = (s, s % 2, pl.multiple_of(((s % 4) // 2) * R, R))
            nxt = jnp.minimum(s + 1, NSTEP - 1)
            w_wait(s, 1)
            start_later(s, 0)
            blk_a(st, nxt)
            if conv == 0:
                w_wait(nxt, 0)
                start_later(s, 1)
            else:
                pl.when(s + 1 < NSTEP)(lambda: w_wait(nxt, 0))
            blk_b(st, nxt)
            return carry

        jax.lax.fori_loop(lo, hi, body, 0)

    conv_loop(0, 1, 4)

    start_next()
    assert next(groups, None) is None
    for cp in small_copies:
        cp.start()

    conv_loop(1, 4, NSTEP)

    for cp in small_copies:
        cp.wait()

    def proj():
        gev[...] = jnp.dot(gv[...], wsm[1], preferred_element_type=F32)
        for _, fn in e2_tasks(0):
            fn()
        for kt in range(NCT):
            _interleave([functools.partial(fe_part, kt)], e2_tasks(kt + 1) if kt + 1 < NCT else [])
        for _, fn in jtasks(0, 0):
            fn()
    block(proj)

    def jbody(a, carry):
        _interleave(jparts(0, a), jtasks(1, a))
        _interleave(jparts(1, a), jtasks(0, a + 1))
        return carry
    jax.lax.fori_loop(0, A - 1, jbody, 0)

    nt_last = T2 - NM * (A - 1)

    def jtail():
        _interleave(jparts(0, A - 1, nt_last), jtasks(1, A - 1, nt_last))
        for p in jparts(1, A - 1, nt_last):
            p()
    block(jtail)

    for b in range(B):
        for a in range(A):
            out_copy(b, a, NM if a + 1 < A else nt_last).wait()
    assert next(flag_ctr) <= NFLAGS


@jax.jit
def pallas_standalone__seq2seq_rnn_t_joint__speech_kernel(
    x: jax.Array,
    w1: jax.Array,
    w2: jax.Array,
    g: jax.Array,
    w_f: jax.Array,
    w_g: jax.Array,
    w_o: jax.Array,
):
    any_spec = pl.BlockSpec(memory_space=pl.ANY)
    out = pl.pallas_call(
        _kernel,
        out_shape=jax.ShapeDtypeStruct((B, T2 * U, D), BF16),
        in_specs=[any_spec] * 7,
        out_specs=any_spec,
        scratch_shapes=[
            pltpu.VMEM((NCT, B, T, LT), BF16),
            pltpu.VMEM((B, NCT, XROWS, LT), F32),
            [pltpu.VMEM((2, NC, R * (PV1 + 4), LT), BF16)] * NCT,
            [pltpu.VMEM((NC, M1, LT), F32)] * NCT,
            pltpu.VMEM((NSTEP, 8, D, D), BF16),
            [pltpu.VMEM((len(MULTI), LT, D), BF16)] * NCT,
            [pltpu.VMEM((len(MULTI), D, LT), BF16)] * NCT,
            pltpu.VMEM((Q2 + 2 * PAD, R, D), F32),
            [pltpu.VMEM((2, NC, R * (PV2 + 4), LT), BF16)] * NCT,
            pltpu.VMEM((NC, M2, D), F32),
            pltpu.VMEM((3, D, D), BF16),
            pltpu.VMEM((B * U, D), BF16),
            pltpu.VMEM((B * U, D), F32),
            [pltpu.VMEM((R * NM, LT), BF16)] * NCT,
            pltpu.VMEM((R * NM, D), F32),
            [pltpu.VMEM((U * NM, D), BF16)] * B,
            pltpu.VMEM((B, T2 * U, D), BF16),
            pltpu.SMEM((NFLAGS,), jnp.int32),
            pltpu.SemaphoreType.DMA((NCT,)),
            pltpu.SemaphoreType.DMA((NCT + 2 * (NSTEP - 1),)),
            pltpu.SemaphoreType.DMA((4,)),
            pltpu.SemaphoreType.DMA((B * A,)),
        ],
        compiler_params=pltpu.CompilerParams(vmem_limit_bytes=120 * 1024 * 1024),
    )(x, w1, w2, g.reshape(B * U, D), w_f, w_g, w_o)
    return out.reshape(B, T2, U, D)
```
